```python
import os as _os
_os.environ.setdefault("JAX_PLATFORMS", "cpu")
import jax
import jax.numpy as jnp

def _softmax(x, axis=-1):
    return jax.nn.softmax(x, axis=axis)
def _gelu(x):
    return jax.nn.gelu(x, approximate=True)
def _silu(x):
    return jax.nn.silu(x)
def _sigmoid(x):
    return jax.nn.sigmoid(x)
def _layernorm(x, axis=-1, eps=1e-5):
    m = jnp.mean(x, axis=axis, keepdims=True)
    v = jnp.var(x, axis=axis, keepdims=True)
    return (x - m) / jnp.sqrt(v + eps)
def _scatter_add(tgt, idx, src, axis=0):
    return tgt.at[idx].add(src)
def _segment_sum(src, seg, n):
    return jax.ops.segment_sum(src, seg, n)
class _Rng:
    def __init__(self, key):
        self._k = key
    def _next(self):
        self._k, sub = jax.random.split(self._k)
        return sub
    def normal(self, shape):
        return jax.random.normal(self._next(), shape, dtype=jnp.bfloat16)
    def randint(self, lo, hi, shape):
        return jax.random.randint(self._next(), shape, lo, hi, dtype=jnp.int32)
    def uniform(self, shape, lo=0.0, hi=1.0):
        return jax.random.uniform(self._next(), shape, jnp.bfloat16, lo, hi)
    def permutation(self, n):
        return jax.random.permutation(self._next(), n)


kernel_name = 'standalone__mha_softmax__near_ridge'

def setup_inputs():
    _rng = _Rng(jax.random.key(int.from_bytes(__import__("os").urandom(4), "little")))
    _w = (lambda a: (lambda t: t.astype(jnp.bfloat16) if jnp.issubdtype(t.dtype, jnp.floating) else t)(jnp.asarray(a)))
    B, H, Sq, Sk, D = 8, 16, 192, 1024, 256
    return {
        "q": _w((lambda *s: _rng.normal(s) * 0.4)(B, H, Sq, D)),
        "k": _w((lambda *s: _rng.normal(s) * 0.4)(B, H, Sk, D)),
        "v": _w((lambda *s: _rng.normal(s) * 0.05)(B, H, Sk, D)),
    }

def reference(q, k, v):
    scale = q.shape[-1] ** -0.5
    scores = jnp.einsum("bhqd,bhkd->bhqk", q, k) * scale
    p = _softmax(scores, axis=-1)
    return jnp.einsum("bhqk,bhkd->bhqd", p, v)
```

```python
import math

import jax
import jax.numpy as jnp
from jax import lax
import jax.experimental.pallas as pl
import jax.experimental.pallas.tpu as pltpu

_NBUF = 4
_WRITE_AT = 3


def _mha_kernel(q_hbm, k_hbm, v_hbm, o_hbm, q_buf, k_buf, v_buf, o_buf, in_sem, out_sem):
    n_heads, _, d = q_hbm.shape
    exp2_scale = (d ** -0.5) * math.log2(math.e)
    n_early = n_heads - _WRITE_AT

    def in_copies(head, slot):
        return (
            (pltpu.make_async_copy(q_hbm.at[head], q_buf.at[slot], in_sem.at[slot, 0]), 0),
            (pltpu.make_async_copy(k_hbm.at[head], k_buf.at[slot], in_sem.at[slot, 1]), 0),
            (pltpu.make_async_copy(v_hbm.at[head], v_buf.at[slot], in_sem.at[slot, 2]), 1),
        )

    def out_copy(start, size, sem):
        return pltpu.make_async_copy(
            o_buf.at[pl.ds(start, size)], o_hbm.at[pl.ds(start, size)], out_sem.at[sem])

    for head in range(_NBUF - 1):
        for copy, priority in in_copies(head, head):
            copy.start(priority=priority)

    def body(head, carry):
        slot = head % _NBUF
        ahead = head + _NBUF - 1

        @pl.when(ahead < n_heads)
        def _():
            for copy, priority in in_copies(ahead, ahead % _NBUF):
                copy.start(priority=priority)

        for copy, _ in in_copies(head, slot):
            copy.wait()

        @pl.when(head == n_early)
        def _():
            out_copy(0, n_early, 0).start()

        s = lax.dot_general(q_buf[slot], k_buf[slot], (((1,), (1,)), ((), ())),
                            preferred_element_type=jnp.float32)
        m = jnp.max(s, axis=-1, keepdims=True)
        p = jnp.exp2((s - m) * exp2_scale)
        l = jnp.sum(p, axis=-1, keepdims=True)
        o = jnp.dot(p.astype(v_buf.dtype), v_buf[slot], preferred_element_type=jnp.float32)
        o_buf[head] = (o * (1.0 / l)).astype(o_buf.dtype)
        return carry

    lax.fori_loop(0, n_heads, body, 0)

    out_copy(n_early, _WRITE_AT, 1).start()
    out_copy(n_early, _WRITE_AT, 1).wait()
    out_copy(0, n_early, 0).wait()


@jax.jit
def pallas_standalone__mha_softmax__near_ridge_kernel(
    q: jax.Array,
    k: jax.Array,
    v: jax.Array,
):
    b, h, sq, d = q.shape
    sk = k.shape[2]
    n_heads = b * h

    out = pl.pallas_call(
        _mha_kernel,
        in_specs=[pl.BlockSpec(memory_space=pl.ANY)] * 3,
        out_specs=pl.BlockSpec(memory_space=pl.ANY),
        out_shape=jax.ShapeDtypeStruct((n_heads, sq, d), q.dtype),
        scratch_shapes=[
            pltpu.VMEM((_NBUF, sq, d), q.dtype),
            pltpu.VMEM((_NBUF, sk, d), k.dtype),
            pltpu.VMEM((_NBUF, sk, d), v.dtype),
            pltpu.VMEM((n_heads, sq, d), q.dtype),
            pltpu.SemaphoreType.DMA((_NBUF, 3)),
            pltpu.SemaphoreType.DMA((2,)),
        ],
        compiler_params=pltpu.CompilerParams(vmem_limit_bytes=64 * 1024 * 1024),
        name="mha_softmax",
    )(q.reshape(n_heads, sq, d), k.reshape(n_heads, sk, d), v.reshape(n_heads, sk, d))
    return out.reshape(b, h, sq, d)
```

```python
import math

import jax
import jax.numpy as jnp
from jax import lax
import jax.experimental.pallas as pl
import jax.experimental.pallas.tpu as pltpu

_GROUP = 4
_HEAD_STRIDE = 4
_WAIT_LAG = 2
_AHEAD = _GROUP - 1 + _WAIT_LAG
_GROUP_BUFS = (_GROUP - 1 + _AHEAD) // _GROUP + 1
_QK_ROWS = 16
_V_ROWS = 32
_KEY_BLOCK = 256
_PINS_PER_ROUND = 3
_PINS_IN_SOFTMAX = 2
_PROLOGUE_NS = 1300
_OUT_ROWS = 32
_OUT_STRIDE = 2048
_TOKEN_ROWS = 16


def _head_of(t):
    group, member = t // _GROUP, t % _GROUP
    return ((group // _HEAD_STRIDE) * _GROUP + member) * _HEAD_STRIDE + group % _HEAD_STRIDE


def _read_units(q_rows, kv_rows):
    pieces = [((r + _QK_ROWS / 2) / q_rows, "q", r, _QK_ROWS) for r in range(0, q_rows, _QK_ROWS)]
    pieces += [((r + _QK_ROWS / 2) / kv_rows, "k", r, _QK_ROWS) for r in range(0, kv_rows, _QK_ROWS)]
    pieces += [(r / kv_rows, "v", r, _V_ROWS) for r in range(0, kv_rows, _V_ROWS)]
    pieces.sort(key=lambda piece: piece[0])
    units, unit = [], []
    for _, name, row, rows in pieces:
        unit.append((name, row, rows))
        if name != "v":
            units.append(unit)
            unit = []
    assert not unit
    return units


def _write_schedule(n_heads, chunks_per_head, n_columns, first_step):
    ready = [first_step] * n_columns
    for t in range(n_heads):
        for c in range(chunks_per_head):
            column = (_head_of(t) * chunks_per_head + c) % n_columns
            ready[column] = max(ready[column], t + 1)
    schedule = {}
    for column in sorted(range(n_columns), key=lambda column: (ready[column], column)):
        schedule.setdefault(ready[column], []).append(column)
    return schedule


def _mha_kernel(q_hbm, k_hbm, v_hbm, o_hbm, in_buf, out_buf, in_sems, out_sem):
    outer, _, _, sq, d = q_hbm.shape
    sk = k_hbm.shape[3]
    n_heads = outer * _GROUP * _HEAD_STRIDE
    n_columns = o_hbm.shape[1]
    chunks_per_head = sq // _OUT_ROWS
    n_rounds = sk // _KEY_BLOCK
    exp2_scale = (d ** -0.5) * math.log2(math.e)

    q_rows, kv_rows = sq // _GROUP, sk // _GROUP
    slice_rows = q_rows + 2 * kv_rows
    source = {"q": q_hbm, "k": k_hbm, "v": v_hbm}
    offset = {"q": 0, "k": q_rows, "v": q_rows + kv_rows}

    def request(s, pieces):
        group, part = s // _GROUP, s % _GROUP
        for name, row, rows in pieces:
            start = pl.multiple_of(part * (q_rows if name == "q" else kv_rows) + row, 16)
            pltpu.make_async_copy(
                source[name].at[group // _HEAD_STRIDE, :, group % _HEAD_STRIDE, pl.ds(start, rows)],
                in_buf.at[group % _GROUP_BUFS, part, :, pl.ds(offset[name] + row, rows)],
                in_sems.at[s % (_WAIT_LAG + 1)],
            ).start(priority=1 if name == "v" else 0)

    def await_slice(s):
        block = in_buf.at[(s // _GROUP) % _GROUP_BUFS, s % _GROUP, :, pl.ds(0, slice_rows)]
        pltpu.make_async_copy(block, block, in_sems.at[s % (_WAIT_LAG + 1)]).wait()

    units = _read_units(q_rows, kv_rows)
    n_pins = 2 * n_rounds * _PINS_PER_ROUND + _PINS_IN_SOFTMAX
    pinned = units[2:]
    pin_pieces = [
        sum(pinned[len(pinned) * i // n_pins:len(pinned) * (i + 1) // n_pins], [])
        for i in range(n_pins)
    ]

    schedule = _write_schedule(
        n_heads, chunks_per_head, n_columns, first_step=n_heads - 2 - _AHEAD + _WAIT_LAG)

    def start_writes(columns):
        for column in columns:
            pltpu.make_async_copy(out_buf.at[:, column], o_hbm.at[:, column], out_sem).start()

    def scheduled_writes(t, lo, hi):
        for step, columns in schedule.items():
            if lo <= step < hi:
                pl.when(t == step)(lambda columns=columns: start_writes(columns))

    def attend(t, prefetch):
        slot, member = (t // _GROUP) % _GROUP_BUFS, t % _GROUP

        def load(name, row, rows):
            per_part = q_rows if name == "q" else kv_rows
            blocks = []
            while rows > 0:
                part, r = divmod(row, per_part)
                n = min(rows, per_part - r)
                blocks.append(in_buf[slot, part, member, pl.ds(offset[name] + r, n)])
                row, rows = row + n, rows - n
            return blocks[0] if len(blocks) == 1 else jnp.concatenate(blocks, axis=0)

        pins = iter(pin_pieces)

        def pin(value, n, i):
            pieces = next(pins)
            if not (prefetch and pieces):
                return
            end = (sq * (i + 1) // n) // 16 * 16
            if value.dtype == jnp.float32:
                token = pltpu.bitcast(value[end - _TOKEN_ROWS // 2:end, -128:], in_buf.dtype)
            else:
                token = value[end - _TOKEN_ROWS:end, -128:]
            in_buf[slot, 0, member, pl.ds(slice_rows, _TOKEN_ROWS), pl.ds(0, 128)] = token
            request(t + _AHEAD, pieces)

        blocks = [(name, r * _KEY_BLOCK, _KEY_BLOCK) for name in "kv" for r in range(n_rounds)]
        rhs = {0: load(*blocks[0]), 1: load(*blocks[1])}

        def pin_round(value, r):
            for i in range(_PINS_PER_ROUND):
                if i == 1 and r + 2 < len(blocks):
                    rhs[r + 2] = load(*blocks[r + 2])
                pin(value, _PINS_PER_ROUND, i)

        q = load("q", 0, sq)
        scores = []
        for r in range(n_rounds):
            scores.append(lax.dot_general(q, rhs.pop(r), (((1,), (1,)), ((), ())),
                                          preferred_element_type=jnp.float32))
            pin_round(scores[-1], r)
        s = jnp.concatenate(scores, axis=1)
        m = jnp.max(s, axis=-1, keepdims=True)
        p = jnp.exp2((s - m) * exp2_scale)
        l = jnp.sum(p, axis=-1, keepdims=True)
        p = p.astype(in_buf.dtype)
        for i in range(_PINS_IN_SOFTMAX):
            pin(p[:, :_KEY_BLOCK], _PINS_IN_SOFTMAX, i)
        o = None
        for r in range(n_rounds):
            pv = jnp.dot(p[:, r * _KEY_BLOCK:(r + 1) * _KEY_BLOCK], rhs.pop(n_rounds + r),
                         preferred_element_type=jnp.float32)
            o = pv if o is None else o + pv
            pin_round(o, n_rounds + r)
        o = (o * (1.0 / l)).astype(out_buf.dtype)
        for c in range(chunks_per_head):
            chunk = _head_of(t) * chunks_per_head + c
            out_buf[chunk // n_columns, chunk % n_columns] = o[c * _OUT_ROWS:(c + 1) * _OUT_ROWS]

    def prologue(s, carry):
        pl.when(s >= _WAIT_LAG)(lambda: await_slice(s - _WAIT_LAG))
        for unit in units:
            request(s, unit)
            pl.delay(_PROLOGUE_NS // len(units))
        return carry

    def steady(t, carry):
        request(t + _AHEAD, units[0])
        await_slice(t + _AHEAD - _WAIT_LAG)
        request(t + _AHEAD, units[1])
        scheduled_writes(t, 0, n_heads - _AHEAD)
        attend(t, prefetch=True)
        return carry

    def drain(t, carry):
        s = t + _AHEAD - _WAIT_LAG
        pl.when(s < n_heads)(lambda: await_slice(s))
        scheduled_writes(t, n_heads - _AHEAD, n_heads)
        attend(t, prefetch=False)
        return carry

    lax.fori_loop(0, _AHEAD, prologue, 0)
    lax.fori_loop(0, n_heads - _AHEAD, steady, 0)
    lax.fori_loop(n_heads - _AHEAD, n_heads, drain, 0)
    start_writes(schedule.get(n_heads, []))
    pltpu.make_async_copy(out_buf, o_hbm, out_sem).wait()


@jax.jit
def pallas_standalone__mha_softmax__near_ridge_kernel(
    q: jax.Array,
    k: jax.Array,
    v: jax.Array,
):
    b, h, sq, d = q.shape
    sk = k.shape[2]
    grouped = (b * h // (_GROUP * _HEAD_STRIDE), _GROUP, _HEAD_STRIDE)
    out_shape = (b * h * sq // _OUT_STRIDE, _OUT_STRIDE // _OUT_ROWS, _OUT_ROWS, d)

    out = pl.pallas_call(
        _mha_kernel,
        in_specs=[pl.BlockSpec(memory_space=pl.ANY)] * 3,
        out_specs=pl.BlockSpec(memory_space=pl.ANY),
        out_shape=jax.ShapeDtypeStruct(out_shape, q.dtype),
        scratch_shapes=[
            pltpu.VMEM((_GROUP_BUFS, _GROUP, _GROUP, (sq + 2 * sk) // _GROUP + _TOKEN_ROWS, d), q.dtype),
            pltpu.VMEM(out_shape, q.dtype),
            pltpu.SemaphoreType.DMA((_WAIT_LAG + 1,)),
            pltpu.SemaphoreType.DMA(()),
        ],
        compiler_params=pltpu.CompilerParams(vmem_limit_bytes=64 * 1024 * 1024),
        name="mha_softmax",
    )(q.reshape(*grouped, sq, d), k.reshape(*grouped, sk, d), v.reshape(*grouped, sk, d))
    return out.reshape(b, h, sq, d)
```

```python
import math

import jax
import jax.numpy as jnp
from jax import lax
import jax.experimental.pallas as pl
import jax.experimental.pallas.tpu as pltpu

_GROUP = 8
_HEAD_STRIDE = 2
_WAIT_LAG = 2
_AHEAD = _GROUP - 1 + _WAIT_LAG
_GROUP_BUFS = 4
_SEM_SLOTS = 4
_QK_ROWS = 8
_V_ROWS = 32
_KEY_BLOCK = 256
_OUT_ROWS = 32
_OUT_STRIDE = 2048
_TOKEN_ROWS = 16
_IDLE_PER_PIECE = 8
_IDLE_BEFORE_WRITES = 40

_PINS = (
    "before_wait", "after_wait", ("k", 1, 128),
    ("s", 0, 16), ("s", 0, 112), ("s", 1, 32), ("s", 1, 128),
    ("s", 2, 48), ("s", 2, 144), ("s", 3, 64), ("s", 3, 160),
    ("p", 0, 16),
    ("o", 0, 80), ("o", 0, 176), ("o", 1, 80), ("o", 1, 176),
    ("o", 2, 96), ("o", 2, 192), ("o", 3, 112),
)


def _div(x, n):
    if isinstance(x, int):
        return x // n
    return lax.shift_right_logical(x, n.bit_length() - 1)


def _mod(x, n):
    if isinstance(x, int):
        return x % n
    return lax.bitwise_and(x, n - 1)


def _head_of(t):
    group, member = _div(t, _GROUP), _mod(t, _GROUP)
    return ((_div(group, _HEAD_STRIDE) * _GROUP + member) * _HEAD_STRIDE
            + _mod(group, _HEAD_STRIDE))


def _slice_pieces(q_rows, kv_rows):
    pieces = [((r + _QK_ROWS / 2) / q_rows, "q", r, _QK_ROWS) for r in range(0, q_rows, _QK_ROWS)]
    pieces += [((r + _QK_ROWS / 2) / kv_rows, "k", r, _QK_ROWS) for r in range(0, kv_rows, _QK_ROWS)]
    pieces += [(r / kv_rows, "v", r, _V_ROWS) for r in range(0, kv_rows, _V_ROWS)]
    pieces.sort(key=lambda piece: piece[0])
    return [piece[1:] for piece in pieces]


def _pinned_pieces(pieces):
    pinned, pending, pins = {}, [], iter(_PINS)
    for piece in pieces:
        pending.append(piece)
        if piece[0] != "v":
            pinned[next(pins)] = pending
            pending = []
    assert not pending
    return pinned


def _write_schedule(n_steps, chunks_per_head, n_columns, first_step):
    ready = [first_step] * n_columns
    for t in range(n_steps):
        for c in range(chunks_per_head):
            column = (_head_of(t) * chunks_per_head + c) % n_columns
            ready[column] = max(ready[column], t + 1)
    schedule = {}
    for column in sorted(range(n_columns), key=lambda column: (ready[column], column)):
        schedule.setdefault(ready[column], []).append(column)
    return schedule


def _mha_kernel(q_hbm, k_hbm, v_hbm, o_hbm, in_buf, out_buf, in_sems, out_sem):
    outer, _, _, sq, d = q_hbm.shape
    sk = k_hbm.shape[3]
    n_steps = outer * _GROUP * _HEAD_STRIDE
    n_columns = o_hbm.shape[1]
    chunks_per_head = sq // _OUT_ROWS
    n_blocks = sk // _KEY_BLOCK
    exp2_scale = (d ** -0.5) * math.log2(math.e)

    source = {"q": q_hbm, "k": k_hbm, "v": v_hbm}
    part_rows = {"q": sq // _GROUP, "k": sk // _GROUP, "v": sk // _GROUP}
    offset = {"q": 0, "k": sq, "v": sq + sk}
    spare = sq + 2 * sk

    def read_copy(s, name, row, rows):
        group = _div(s, _GROUP)
        start = _mod(s, _GROUP) * part_rows[name] + row
        return pltpu.make_async_copy(
            source[name].at[_div(group, _HEAD_STRIDE), :, _mod(group, _HEAD_STRIDE),
                            pl.ds(pl.multiple_of(start, 8), rows)],
            in_buf.at[_mod(group, _GROUP_BUFS), :,
                      pl.ds(pl.multiple_of(offset[name] + start, 8), rows)],
            in_sems.at["qkv".index(name), _mod(s, _SEM_SLOTS)])

    def request(s, pieces):
        for name, row, rows in pieces:
            read_copy(s, name, row, rows).start(priority=1 if name == "v" else 0)

    def await_slice(s):
        for name in "qkv":
            read_copy(s, name, 0, part_rows[name]).wait()

    def store_token(i, value):
        in_buf[i // _GROUP, i % _GROUP, pl.ds(spare, _TOKEN_ROWS), pl.ds(0, 128)] = (
            value.astype(in_buf.dtype))

    def idle(n):
        def step(_, carry):
            store_token(0, jnp.zeros((_TOKEN_ROWS, 128), in_buf.dtype))
            return carry
        lax.fori_loop(0, n, step, 0)

    pieces = _slice_pieces(part_rows["q"], part_rows["k"])
    pinned = _pinned_pieces(pieces)

    first_write = n_steps - 2 - _AHEAD + _WAIT_LAG
    assert first_write >= n_steps - _AHEAD
    schedule = _write_schedule(n_steps, chunks_per_head, n_columns, first_write)

    def start_writes(columns):
        for column in columns:
            pltpu.make_async_copy(out_buf.at[:, column], o_hbm.at[:, column], out_sem).start()

    def attend(t, prefetch):
        slot, member = _mod(_div(t, _GROUP), _GROUP_BUFS), _mod(t, _GROUP)

        def load(name, row, rows):
            return in_buf[slot, member, pl.ds(offset[name] + row, rows)]

        def pin(kind, block, value):
            if not prefetch:
                return
            for i, key in enumerate(_PINS):
                if key in pinned and key[:2] == (kind, block):
                    store_token(i, value[key[2] - _TOKEN_ROWS:key[2], -128:])
                    request(t + _AHEAD, pinned[key])

        blocks = [(name, i * _KEY_BLOCK, _KEY_BLOCK) for name in "kv" for i in range(n_blocks)]
        q = load("q", 0, sq)
        rhs = [load(*blocks[0])]
        half = load("k", _KEY_BLOCK, _KEY_BLOCK // 2)
        pin("k", 1, half)
        rhs.append(jnp.concatenate(
            [half, load("k", _KEY_BLOCK * 3 // 2, _KEY_BLOCK // 2)], axis=0))

        scores = []
        for i in range(n_blocks):
            scores.append(lax.dot_general(q, rhs[i], (((1,), (1,)), ((), ())),
                                          preferred_element_type=jnp.float32))
            pin("s", i, scores[i])
            rhs.append(load(*blocks[i + 2]))
        s = jnp.concatenate(scores, axis=1)
        m = jnp.max(s, axis=-1, keepdims=True)
        p = jnp.exp2((s - m) * exp2_scale)
        l = jnp.sum(p, axis=-1, keepdims=True)

        o = None
        for i in range(n_blocks):
            p_block = p[:, i * _KEY_BLOCK:(i + 1) * _KEY_BLOCK]
            pin("p", i, p_block)
            pv = jnp.dot(p_block.astype(in_buf.dtype), rhs[n_blocks + i],
                         preferred_element_type=jnp.float32)
            o = pv if o is None else o + pv
            pin("o", i, o)
            if n_blocks + i + 2 < len(blocks):
                rhs.append(load(*blocks[n_blocks + i + 2]))
        o = (o * (1.0 / l)).astype(out_buf.dtype)

        for c in range(chunks_per_head):
            chunk = _head_of(t) * chunks_per_head + c
            out_buf[_div(chunk, n_columns), _mod(chunk, n_columns)] = (
                o[c * _OUT_ROWS:(c + 1) * _OUT_ROWS])

    def fill(s, carry):
        pl.when(s >= _WAIT_LAG)(lambda: await_slice(s - _WAIT_LAG))
        request(s, [piece for piece in pieces if piece[0] == "v"])
        for piece in pieces:
            if piece[0] != "v":
                request(s, [piece])
                idle(_IDLE_PER_PIECE)
        return carry

    def steady(t, carry):
        request(t + _AHEAD, pinned["before_wait"])
        await_slice(t + _AHEAD - _WAIT_LAG)
        request(t + _AHEAD, pinned["after_wait"])
        attend(t, prefetch=True)
        return carry

    def drain(t, carry):
        s = t + _AHEAD - _WAIT_LAG
        pl.when(s < n_steps)(lambda: await_slice(s))
        pl.when(t == first_write)(lambda: idle(_IDLE_BEFORE_WRITES))
        for step, columns in schedule.items():
            if step < n_steps:
                pl.when(t == step)(lambda columns=columns: start_writes(columns))
        attend(t, prefetch=False)
        return carry

    lax.fori_loop(0, _AHEAD, fill, 0)
    lax.fori_loop(0, n_steps - _AHEAD, steady, 0)
    lax.fori_loop(n_steps - _AHEAD, n_steps, drain, 0)
    start_writes(schedule.get(n_steps, []))
    pltpu.make_async_copy(out_buf, o_hbm, out_sem).wait()


@jax.jit
def pallas_standalone__mha_softmax__near_ridge_kernel(
    q: jax.Array,
    k: jax.Array,
    v: jax.Array,
):
    b, h, sq, d = q.shape
    sk = k.shape[2]
    assert (b * h) % (_GROUP * _HEAD_STRIDE) == 0 and (b * h * sq) % _OUT_STRIDE == 0
    assert sq % (_GROUP * _QK_ROWS) == 0 and sq % _OUT_ROWS == 0
    assert sk % (_GROUP * _V_ROWS) == 0 and sk % _KEY_BLOCK == 0
    grouped = (b * h // (_GROUP * _HEAD_STRIDE), _GROUP, _HEAD_STRIDE)
    out_shape = (b * h * sq // _OUT_STRIDE, _OUT_STRIDE // _OUT_ROWS, _OUT_ROWS, d)

    out = pl.pallas_call(
        _mha_kernel,
        in_specs=[pl.BlockSpec(memory_space=pl.ANY)] * 3,
        out_specs=pl.BlockSpec(memory_space=pl.ANY),
        out_shape=jax.ShapeDtypeStruct(out_shape, q.dtype),
        scratch_shapes=[
            pltpu.VMEM((_GROUP_BUFS, _GROUP, sq + 2 * sk + _TOKEN_ROWS, d), q.dtype),
            pltpu.VMEM(out_shape, q.dtype),
            pltpu.SemaphoreType.DMA((3, _SEM_SLOTS)),
            pltpu.SemaphoreType.DMA(()),
        ],
        compiler_params=pltpu.CompilerParams(vmem_limit_bytes=72 * 1024 * 1024),
        name="mha_softmax",
    )(q.reshape(*grouped, sq, d), k.reshape(*grouped, sk, d), v.reshape(*grouped, sk, d))
    return out.reshape(b, h, sq, d)
```

```python
import functools
import math

import jax
import jax.numpy as jnp
from jax import lax
import jax.experimental.pallas as pl
import jax.experimental.pallas.tpu as pltpu

_GROUP = 8
_HEAD_STRIDE = 2
_WAIT_LAG = 2
_AHEAD = _GROUP - 1 + _WAIT_LAG
_GROUP_BUFS = 4
_SEM_SLOTS = 4
_QK_ROWS = 8
_V_ROWS = 32
_KEY_BLOCK = 256
_OUT_ROWS = 32
_OUT_STRIDE = 2048
_TOKEN_ROWS = 16
_IDLE_PER_PIECE = 8
_IDLE_BEFORE_WRITES = 40

_PINS = (
    "before_wait", "after_wait", ("k", 1, 128),
    ("s", 0, 16), ("s", 0, 112), ("s", 1, 32), ("s", 1, 128),
    ("s", 2, 48), ("s", 2, 144), ("s", 3, 64), ("s", 3, 160),
    ("p", 0, 16),
    ("o", 0, 80), ("o", 0, 176), ("o", 1, 80), ("o", 1, 176),
    ("o", 2, 96), ("o", 2, 192), ("o", 3, 112),
)


def _div(x, n):
    if isinstance(x, int):
        return x // n
    return lax.shift_right_logical(x, n.bit_length() - 1)


def _mod(x, n):
    if isinstance(x, int):
        return x % n
    return lax.bitwise_and(x, n - 1)


def _head_of(t):
    group, member = _div(t, _GROUP), _mod(t, _GROUP)
    return ((_div(group, _HEAD_STRIDE) * _GROUP + member) * _HEAD_STRIDE
            + _mod(group, _HEAD_STRIDE))


def _slice_pieces(q_rows, kv_rows):
    pieces = [((r + _QK_ROWS / 2) / q_rows, "q", r, _QK_ROWS) for r in range(0, q_rows, _QK_ROWS)]
    pieces += [((r + _QK_ROWS / 2) / kv_rows, "k", r, _QK_ROWS) for r in range(0, kv_rows, _QK_ROWS)]
    pieces += [(r / kv_rows, "v", r, _V_ROWS) for r in range(0, kv_rows, _V_ROWS)]
    pieces.sort(key=lambda piece: piece[0])
    return [piece[1:] for piece in pieces]


def _pinned_pieces(pieces):
    pinned, pending, pins = {}, [], iter(_PINS)
    for piece in pieces:
        pending.append(piece)
        if piece[0] != "v":
            pinned[next(pins)] = pending
            pending = []
    assert not pending
    return pinned


def _write_schedule(n_steps, chunks_per_head, n_columns, first_step):
    ready = [first_step] * n_columns
    for t in range(n_steps):
        for c in range(chunks_per_head):
            column = (_head_of(t) * chunks_per_head + c) % n_columns
            ready[column] = max(ready[column], t + 1)
    schedule = {}
    for column in sorted(range(n_columns), key=lambda column: (ready[column], column)):
        schedule.setdefault(ready[column], []).append(column)
    return schedule


def _attend_all(q_hbm, k_hbm, v_hbm, o_hbm, in_buf, out_buf, out_sem, in_sems):
    outer, _, _, sq, d = q_hbm.shape
    sk = k_hbm.shape[3]
    n_steps = outer * _GROUP * _HEAD_STRIDE
    n_columns = o_hbm.shape[1]
    chunks_per_head = sq // _OUT_ROWS
    n_blocks = sk // _KEY_BLOCK
    exp2_scale = (d ** -0.5) * math.log2(math.e)

    source = {"q": q_hbm, "k": k_hbm, "v": v_hbm}
    part_rows = {"q": sq // _GROUP, "k": sk // _GROUP, "v": sk // _GROUP}
    offset = {"q": 0, "k": sq, "v": sq + sk}
    spare = sq + 2 * sk
    pieces = _slice_pieces(part_rows["q"], part_rows["k"])
    pinned = _pinned_pieces(pieces)

    def read_copy(s, name, row, rows):
        group = _div(s, _GROUP)
        start = _mod(s, _GROUP) * part_rows[name] + row
        return pltpu.make_async_copy(
            source[name].at[_div(group, _HEAD_STRIDE), :, _mod(group, _HEAD_STRIDE),
                            pl.ds(pl.multiple_of(start, 8), rows)],
            in_buf.at[_mod(group, _GROUP_BUFS), :,
                      pl.ds(pl.multiple_of(offset[name] + start, 8), rows)],
            in_sems.at[_mod(s, _SEM_SLOTS)])

    def request(s, pieces):
        for name, row, rows in pieces:
            read_copy(s, name, row, rows).start(priority=1 if name == "v" else 0)

    def await_slice(s):
        for piece in pieces:
            read_copy(s, *piece).wait()

    def store_token(i, value):
        in_buf[i // _GROUP, i % _GROUP, pl.ds(spare, _TOKEN_ROWS), pl.ds(0, 128)] = (
            value.astype(in_buf.dtype))

    def idle(n):
        def step(_, carry):
            store_token(0, jnp.zeros((_TOKEN_ROWS, 128), in_buf.dtype))
            return carry
        lax.fori_loop(0, n, step, 0)

    first_write = n_steps - 2 - _AHEAD + _WAIT_LAG
    assert first_write >= n_steps - _AHEAD
    schedule = _write_schedule(n_steps, chunks_per_head, n_columns, first_write)

    def start_writes(columns):
        for column in columns:
            pltpu.make_async_copy(out_buf.at[:, column], o_hbm.at[:, column], out_sem).start()

    def attend(t, prefetch):
        slot, member = _mod(_div(t, _GROUP), _GROUP_BUFS), _mod(t, _GROUP)

        def load(name, row, rows):
            return in_buf[slot, member, pl.ds(offset[name] + row, rows)]

        def pin(kind, block, value):
            if not prefetch:
                return
            for i, key in enumerate(_PINS):
                if key in pinned and key[:2] == (kind, block):
                    store_token(i, value[key[2] - _TOKEN_ROWS:key[2], -128:])
                    request(t + _AHEAD, pinned[key])

        blocks = [(name, i * _KEY_BLOCK, _KEY_BLOCK) for name in "kv" for i in range(n_blocks)]
        q = load("q", 0, sq)
        rhs = [load(*blocks[0])]
        half = load("k", _KEY_BLOCK, _KEY_BLOCK // 2)
        pin("k", 1, half)
        rhs.append(jnp.concatenate(
            [half, load("k", _KEY_BLOCK * 3 // 2, _KEY_BLOCK // 2)], axis=0))

        scores = []
        for i in range(n_blocks):
            scores.append(lax.dot_general(q, rhs[i], (((1,), (1,)), ((), ())),
                                          preferred_element_type=jnp.float32))
            pin("s", i, scores[i])
            rhs.append(load(*blocks[i + 2]))
        s = jnp.concatenate(scores, axis=1)
        m = jnp.max(s, axis=-1, keepdims=True)
        p = jnp.exp2((s - m) * exp2_scale)
        l = jnp.sum(p, axis=-1, keepdims=True)

        o = None
        for i in range(n_blocks):
            p_block = p[:, i * _KEY_BLOCK:(i + 1) * _KEY_BLOCK]
            pin("p", i, p_block)
            pv = jnp.dot(p_block.astype(in_buf.dtype), rhs[n_blocks + i],
                         preferred_element_type=jnp.float32)
            o = pv if o is None else o + pv
            pin("o", i, o)
            if n_blocks + i + 2 < len(blocks):
                rhs.append(load(*blocks[n_blocks + i + 2]))
        o = (o * (1.0 / l)).astype(out_buf.dtype)

        for c in range(chunks_per_head):
            chunk = _head_of(t) * chunks_per_head + c
            out_buf[_div(chunk, n_columns), _mod(chunk, n_columns)] = (
                o[c * _OUT_ROWS:(c + 1) * _OUT_ROWS])

    def fill(s, carry):
        pl.when(s >= _WAIT_LAG)(lambda: await_slice(s - _WAIT_LAG))
        request(s, [piece for piece in pieces if piece[0] == "v"])
        for piece in pieces:
            if piece[0] != "v":
                request(s, [piece])
                idle(_IDLE_PER_PIECE)
        return carry

    def steady(t, carry):
        request(t + _AHEAD, pinned["before_wait"])
        await_slice(t + _AHEAD - _WAIT_LAG)
        request(t + _AHEAD, pinned["after_wait"])
        attend(t, prefetch=True)
        return carry

    def drain(t, carry):
        s = t + _AHEAD - _WAIT_LAG
        pl.when(s < n_steps)(lambda: await_slice(s))
        pl.when(t == first_write)(lambda: idle(_IDLE_BEFORE_WRITES))
        for step, columns in schedule.items():
            if step < n_steps:
                pl.when(t == step)(lambda columns=columns: start_writes(columns))
        attend(t, prefetch=False)
        return carry

    lax.fori_loop(0, _AHEAD, fill, 0)
    lax.fori_loop(0, n_steps - _AHEAD, steady, 0)
    lax.fori_loop(n_steps - _AHEAD, n_steps, drain, 0)
    start_writes(schedule.get(n_steps, []))


def _mha_kernel(q_hbm, k_hbm, v_hbm, o_hbm, in_buf, out_buf, out_sem):
    pl.run_scoped(
        functools.partial(_attend_all, q_hbm, k_hbm, v_hbm, o_hbm, in_buf, out_buf, out_sem),
        pltpu.SemaphoreType.DMA((_SEM_SLOTS,)))
    pltpu.make_async_copy(out_buf, o_hbm, out_sem).wait()


@jax.jit
def pallas_standalone__mha_softmax__near_ridge_kernel(
    q: jax.Array,
    k: jax.Array,
    v: jax.Array,
):
    b, h, sq, d = q.shape
    sk = k.shape[2]
    assert (b * h) % (_GROUP * _HEAD_STRIDE) == 0 and (b * h * sq) % _OUT_STRIDE == 0
    assert sq % (_GROUP * _QK_ROWS) == 0 and sq % _OUT_ROWS == 0
    assert sk % (_GROUP * _V_ROWS) == 0 and sk % _KEY_BLOCK == 0
    grouped = (b * h // (_GROUP * _HEAD_STRIDE), _GROUP, _HEAD_STRIDE)
    out_shape = (b * h * sq // _OUT_STRIDE, _OUT_STRIDE // _OUT_ROWS, _OUT_ROWS, d)

    out = pl.pallas_call(
        _mha_kernel,
        in_specs=[pl.BlockSpec(memory_space=pl.ANY)] * 3,
        out_specs=pl.BlockSpec(memory_space=pl.ANY),
        out_shape=jax.ShapeDtypeStruct(out_shape, q.dtype),
        scratch_shapes=[
            pltpu.VMEM((_GROUP_BUFS, _GROUP, sq + 2 * sk + _TOKEN_ROWS, d), q.dtype),
            pltpu.VMEM(out_shape, q.dtype),
            pltpu.SemaphoreType.DMA(()),
        ],
        compiler_params=pltpu.CompilerParams(vmem_limit_bytes=72 * 1024 * 1024),
        name="mha_softmax",
    )(q.reshape(*grouped, sq, d), k.reshape(*grouped, sk, d), v.reshape(*grouped, sk, d))
    return out.reshape(b, h, sq, d)
```

```python
import functools
import math

import jax
import jax.numpy as jnp
from jax import lax
import jax.experimental.pallas as pl
import jax.experimental.pallas.tpu as pltpu

_GROUP = 8
_HEAD_STRIDE = 2
_WAIT_LAG = 2
_AHEAD = _GROUP - 1 + _WAIT_LAG
_GROUP_BUFS = 4
_SEM_SLOTS = 4
_QK_ROWS = 8
_V_ROWS = 32
_KEY_BLOCK = 256
_OUT_ROWS = 32
_OUT_STRIDE = 2048
_TOKEN_ROWS = 16
_IDLE_PER_PIECE = 8
_IDLE_BEFORE_WRITES = 40

_PINS = (
    "before_wait", "after_wait", ("k", 1, 128),
    ("s", 0, 16), ("s", 0, 112), ("s", 1, 32), ("s", 1, 128),
    ("s", 2, 48), ("s", 2, 144), ("s", 3, 64), ("s", 3, 160),
    ("p", 0, 16),
    ("o", 0, 80), ("o", 0, 176), ("o", 1, 80), ("o", 1, 176),
    ("o", 2, 96), ("o", 2, 192), ("o", 3, 112),
)


def _div(x, n):
    if isinstance(x, int):
        return x // n
    return lax.shift_right_logical(x, n.bit_length() - 1)


def _mod(x, n):
    if isinstance(x, int):
        return x % n
    return lax.bitwise_and(x, n - 1)


def _head_of(t):
    group, member = _div(t, _GROUP), _mod(t, _GROUP)
    return ((_div(group, _HEAD_STRIDE) * _GROUP + member) * _HEAD_STRIDE
            + _mod(group, _HEAD_STRIDE))


def _slice_pieces(q_rows, kv_rows):
    pieces = [((r + _QK_ROWS / 2) / q_rows, "q", r, _QK_ROWS) for r in range(0, q_rows, _QK_ROWS)]
    pieces += [((r + _QK_ROWS / 2) / kv_rows, "k", r, _QK_ROWS) for r in range(0, kv_rows, _QK_ROWS)]
    pieces += [(r / kv_rows, "v", r, _V_ROWS) for r in range(0, kv_rows, _V_ROWS)]
    pieces.sort(key=lambda piece: piece[0])
    return [piece[1:] for piece in pieces]


def _pinned_pieces(pieces):
    pinned, pending, pins = {}, [], iter(_PINS)
    for piece in pieces:
        pending.append(piece)
        if piece[0] != "v":
            pinned[next(pins)] = pending
            pending = []
    assert not pending and len(pinned) == len(_PINS)
    return pinned


def _write_schedule(n_steps, chunks_per_head, n_columns, first_step):
    ready = [first_step] * n_columns
    for t in range(n_steps):
        for c in range(chunks_per_head):
            column = (_head_of(t) * chunks_per_head + c) % n_columns
            ready[column] = max(ready[column], t + 1)
    schedule = {}
    for column in sorted(range(n_columns), key=lambda column: (ready[column], column)):
        schedule.setdefault(ready[column], []).append(column)
    return schedule


def _attend_all(q_hbm, k_hbm, v_hbm, o_hbm, in_buf, out_buf, out_sem, in_sems):
    outer, _, _, sq, d = q_hbm.shape
    sk = k_hbm.shape[3]
    n_steps = outer * _GROUP * _HEAD_STRIDE
    n_columns = o_hbm.shape[1]
    chunks_per_head = sq // _OUT_ROWS
    n_blocks = sk // _KEY_BLOCK
    exp2_scale = (d ** -0.5) * math.log2(math.e)

    source = {"q": q_hbm, "k": k_hbm, "v": v_hbm}
    part_rows = {"q": sq // _GROUP, "k": sk // _GROUP, "v": sk // _GROUP}
    offset = {"q": 0, "k": sq, "v": sq + sk}
    spare = sq + 2 * sk
    pieces = _slice_pieces(part_rows["q"], part_rows["k"])
    pinned = _pinned_pieces(pieces)

    def read_copy(s, name, row, rows):
        group = _div(s, _GROUP)
        start = _mod(s, _GROUP) * part_rows[name] + row
        return pltpu.make_async_copy(
            source[name].at[_div(group, _HEAD_STRIDE), :, _mod(group, _HEAD_STRIDE),
                            pl.ds(pl.multiple_of(start, 8), rows)],
            in_buf.at[_mod(group, _GROUP_BUFS), :,
                      pl.ds(pl.multiple_of(offset[name] + start, 8), rows)],
            in_sems.at[_mod(s, _SEM_SLOTS)])

    def request(s, pieces):
        for name, row, rows in pieces:
            read_copy(s, name, row, rows).start(priority=1 if name == "v" else 0)

    def await_slice(s):
        for piece in pieces:
            read_copy(s, *piece).wait()

    def store_token(i, value):
        in_buf[i // _GROUP, i % _GROUP, pl.ds(spare, _TOKEN_ROWS), pl.ds(0, 128)] = (
            value.astype(in_buf.dtype))

    def idle(n):
        def step(_, carry):
            store_token(0, jnp.zeros((_TOKEN_ROWS, 128), in_buf.dtype))
            return carry
        lax.fori_loop(0, n, step, 0)

    first_write = n_steps - 2 - _AHEAD + _WAIT_LAG
    assert first_write >= n_steps - _AHEAD
    schedule = _write_schedule(n_steps, chunks_per_head, n_columns, first_write)

    def start_writes(columns):
        for column in columns:
            pltpu.make_async_copy(out_buf.at[:, column], o_hbm.at[:, column], out_sem).start()

    def attend(t, prefetch):
        slot, member = _mod(_div(t, _GROUP), _GROUP_BUFS), _mod(t, _GROUP)

        def load(name, row, rows):
            return in_buf[slot, member, pl.ds(offset[name] + row, rows)]

        def pin(kind, block, value):
            if not prefetch:
                return
            for i, key in enumerate(_PINS):
                if key[:2] == (kind, block):
                    store_token(i, value[key[2] - _TOKEN_ROWS:key[2], -128:])
                    request(t + _AHEAD, pinned[key])

        blocks = [(name, i * _KEY_BLOCK, _KEY_BLOCK) for name in "kv" for i in range(n_blocks)]
        q = load("q", 0, sq)
        rhs = [load(*blocks[0])]
        half = load("k", _KEY_BLOCK, _KEY_BLOCK // 2)
        pin("k", 1, half)
        rhs.append(jnp.concatenate(
            [half, load("k", _KEY_BLOCK * 3 // 2, _KEY_BLOCK // 2)], axis=0))

        scores = []
        for i in range(n_blocks):
            scores.append(lax.dot_general(q, rhs[i], (((1,), (1,)), ((), ())),
                                          preferred_element_type=jnp.float32))
            pin("s", i, scores[i])
            rhs.append(load(*blocks[i + 2]))
        s = jnp.concatenate(scores, axis=1)
        m = jnp.max(s, axis=-1, keepdims=True)
        p = jnp.exp2((s - m) * exp2_scale)
        l = jnp.sum(p, axis=-1, keepdims=True)

        o = None
        for i in range(n_blocks):
            p_block = p[:, i * _KEY_BLOCK:(i + 1) * _KEY_BLOCK]
            pin("p", i, p_block)
            pv = jnp.dot(p_block.astype(in_buf.dtype), rhs[n_blocks + i],
                         preferred_element_type=jnp.float32)
            o = pv if o is None else o + pv
            pin("o", i, o)
            if n_blocks + i + 2 < len(blocks):
                rhs.append(load(*blocks[n_blocks + i + 2]))
        o = (o * (1.0 / l)).astype(out_buf.dtype)

        for c in range(chunks_per_head):
            chunk = _head_of(t) * chunks_per_head + c
            out_buf[_div(chunk, n_columns), _mod(chunk, n_columns)] = (
                o[c * _OUT_ROWS:(c + 1) * _OUT_ROWS])

    def fill(s, carry):
        pl.when(s >= _WAIT_LAG)(lambda: await_slice(s - _WAIT_LAG))
        request(s, [piece for piece in pieces if piece[0] == "v"])
        for piece in pieces:
            if piece[0] != "v":
                request(s, [piece])
                idle(_IDLE_PER_PIECE)
        return carry

    def steady(t, carry):
        request(t + _AHEAD, pinned["before_wait"])
        await_slice(t + _AHEAD - _WAIT_LAG)
        request(t + _AHEAD, pinned["after_wait"])
        attend(t, prefetch=True)
        return carry

    def drain(t, carry):
        s = t + _AHEAD - _WAIT_LAG
        pl.when(s < n_steps)(lambda: await_slice(s))
        pl.when(t == first_write)(lambda: idle(_IDLE_BEFORE_WRITES))
        for step, columns in schedule.items():
            if step < n_steps:
                pl.when(t == step)(lambda columns=columns: start_writes(columns))
        attend(t, prefetch=False)
        return carry

    lax.fori_loop(0, _AHEAD, fill, 0)
    lax.fori_loop(0, n_steps - _AHEAD, steady, 0)
    lax.fori_loop(n_steps - _AHEAD, n_steps, drain, 0)
    start_writes(schedule.get(n_steps, []))


def _mha_kernel(q_hbm, k_hbm, v_hbm, o_hbm, in_buf, out_buf, out_sem):
    pl.run_scoped(
        functools.partial(_attend_all, q_hbm, k_hbm, v_hbm, o_hbm, in_buf, out_buf, out_sem),
        pltpu.SemaphoreType.DMA((_SEM_SLOTS,)))
    pltpu.make_async_copy(out_buf, o_hbm, out_sem).wait()


@jax.jit
def pallas_standalone__mha_softmax__near_ridge_kernel(
    q: jax.Array,
    k: jax.Array,
    v: jax.Array,
):
    b, h, sq, d = q.shape
    sk = k.shape[2]
    assert (sq, sk) == (192, 1024), "_PINS is laid out for these sequence lengths"
    assert (b * h) % (_GROUP * _HEAD_STRIDE) == 0 and (b * h * sq) % _OUT_STRIDE == 0
    grouped = (b * h // (_GROUP * _HEAD_STRIDE), _GROUP, _HEAD_STRIDE)
    out_shape = (b * h * sq // _OUT_STRIDE, _OUT_STRIDE // _OUT_ROWS, _OUT_ROWS, d)

    out = pl.pallas_call(
        _mha_kernel,
        in_specs=[pl.BlockSpec(memory_space=pl.ANY)] * 3,
        out_specs=pl.BlockSpec(memory_space=pl.ANY),
        out_shape=jax.ShapeDtypeStruct(out_shape, q.dtype),
        scratch_shapes=[
            pltpu.VMEM((_GROUP_BUFS, _GROUP, sq + 2 * sk + _TOKEN_ROWS, d), q.dtype),
            pltpu.VMEM(out_shape, q.dtype),
            pltpu.SemaphoreType.DMA(()),
        ],
        compiler_params=pltpu.CompilerParams(vmem_limit_bytes=72 * 1024 * 1024),
        name="mha_softmax",
    )(q.reshape(*grouped, sq, d), k.reshape(*grouped, sk, d), v.reshape(*grouped, sk, d))
    return out.reshape(b, h, sq, d)
```
